```python
import jax
import jax.numpy as jnp

def _softmax(x, axis=-1):
    return jax.nn.softmax(x, axis=axis)
def _gelu(x):
    return jax.nn.gelu(x, approximate=True)
def _silu(x):
    return jax.nn.silu(x)
def _sigmoid(x):
    return jax.nn.sigmoid(x)
def _layernorm(x, axis=-1, eps=1e-5):
    m = jnp.mean(x, axis=axis, keepdims=True)
    v = jnp.var(x, axis=axis, keepdims=True)
    return (x - m) / jnp.sqrt(v + eps)
def _scatter_add(tgt, idx, src, axis=0):
    return tgt.at[idx].add(src)
def _segment_sum(src, seg, n):
    return jax.ops.segment_sum(src, seg, n)
class _Rng:
    def __init__(self, key):
        self._k = key
    def _next(self):
        self._k, sub = jax.random.split(self._k)
        return sub
    def normal(self, shape):
        return jax.random.normal(self._next(), shape, dtype=jnp.bfloat16)
    def randint(self, lo, hi, shape):
        return jax.random.randint(self._next(), shape, lo, hi, dtype=jnp.int32)
    def uniform(self, shape, lo=0.0, hi=1.0):
        return jax.random.uniform(self._next(), shape, jnp.bfloat16, lo, hi)
    def permutation(self, n):
        return jax.random.permutation(self._next(), n)


kernel_name = 'standalone__gqa_softmax__near_ridge'

def setup_inputs():
    _rng = _Rng(jax.random.key(int.from_bytes(__import__("os").urandom(4), "little")))
    _w = (lambda a: (lambda t: t.astype(jnp.bfloat16) if jnp.issubdtype(t.dtype, jnp.floating) else t)(jnp.asarray(a)))
    B, Hq, Hkv, Sq, Sk, D = 16, 32, 32, 848, 512, 192
    return {
        "q": _w((lambda *s: _rng.normal(s) * 0.05)(B, Hq, Sq, D)),
        "k": _w((lambda *s: _rng.normal(s) * 0.05)(B, Hkv, Sk, D)),
        "v": _w((lambda *s: _rng.normal(s) * 0.05)(B, Hkv, Sk, D)),
    }

def reference(q, k, v):
    B, Hq, Sq, D = q.shape
    Hkv = k.shape[1]
    rep = Hq // Hkv
    k = jnp.repeat(k, rep, axis=1)
    v = jnp.repeat(v, rep, axis=1)
    scale = D ** -0.5
    scores = jnp.einsum("bhqd,bhkd->bhqk", q, k) * scale
    p = _softmax(scores, axis=-1)
    return jnp.einsum("bhqk,bhkd->bhqd", p, v)
```

```python
import jax
import jax.numpy as jnp
import jax.experimental.pallas as pl
import jax.experimental.pallas.tpu as pltpu
import ml_dtypes
import numpy as np

_HEADS_PER_STEP = 4


@jax.jit
def pallas_standalone__gqa_softmax__near_ridge_kernel(
    q: jax.Array,
    k: jax.Array,
    v: jax.Array,
):
    B, Hq, Sq, D = q.shape
    Hkv, Sk = k.shape[1], k.shape[2]
    assert Hq == Hkv
    hb = _HEADS_PER_STEP
    scale = float(np.asarray(D ** -0.5, dtype=ml_dtypes.bfloat16))
    c = scale * float(np.log2(np.e))

    qT = jnp.swapaxes(q, 2, 3).reshape(B * Hq, D, Sq)
    kT = jnp.swapaxes(k, 2, 3).reshape(B * Hkv, D, Sk)
    vT = jnp.swapaxes(v, 2, 3).reshape(B * Hkv, D, Sk)

    def kernel_function(q_ref, k_ref, v_ref, o_ref):
        for h in range(hb):
            s = jax.lax.dot_general(
                k_ref[h], q_ref[h], (((0,), (0,)), ((), ())),
                preferred_element_type=jnp.float32)
            m = jnp.max(s, axis=0, keepdims=True)
            p = jnp.exp2((s - m) * c)
            l = jnp.sum(p, axis=0, keepdims=True)
            o = jnp.dot(v_ref[h], p.astype(v_ref.dtype),
                        preferred_element_type=jnp.float32)
            o_ref[h] = (o * (1.0 / l)).astype(o_ref.dtype)

    oT = pl.pallas_call(
        kernel_function,
        grid=(B * Hq // hb,),
        in_specs=[
            pl.BlockSpec((hb, D, Sq), lambda i: (i, 0, 0)),
            pl.BlockSpec((hb, D, Sk), lambda i: (i, 0, 0)),
            pl.BlockSpec((hb, D, Sk), lambda i: (i, 0, 0)),
        ],
        out_specs=pl.BlockSpec((hb, D, Sq), lambda i: (i, 0, 0)),
        out_shape=jax.ShapeDtypeStruct((B * Hq, D, Sq), q.dtype),
        compiler_params=pltpu.CompilerParams(
            dimension_semantics=("parallel",),
            vmem_limit_bytes=100 * 1024 * 1024),
    )(qT, kT, vT)
    return jnp.swapaxes(oT.reshape(B, Hq, D, Sq), 2, 3)
```

```python
import jax
import jax.numpy as jnp
import jax.experimental.pallas as pl
import jax.experimental.pallas.tpu as pltpu
import ml_dtypes
import numpy as np

_HEADS = 8
_LANES = 128
_S_SLOTS = 4
_K_SLOTS = 2


def _dot(a, b):
    return jnp.dot(a, b, preferred_element_type=jnp.float32)


def _fold(x, rows=8):
    return jnp.sum(x.reshape(-1, rows, x.shape[-1]), axis=0)


@jax.jit
def pallas_standalone__gqa_softmax__near_ridge_kernel(
    q: jax.Array,
    k: jax.Array,
    v: jax.Array,
):
    B, H, Sq, D = q.shape
    Sk = k.shape[2]
    assert k.shape == v.shape == (B, H, Sk, D)
    assert q.dtype == k.dtype == v.dtype == jnp.bfloat16
    assert D == 192 and Sk == 512 and (B * H) % _HEADS == 0
    f32, bf16, u32 = jnp.float32, jnp.bfloat16, jnp.uint32

    scale = float(np.asarray(D**-0.5, dtype=ml_dtypes.bfloat16))
    log2_scale = scale * float(np.log2(np.e))

    n_blocks = B * H // _HEADS
    tiles = pl.cdiv(Sq, _LANES)
    units = _HEADS * tiles
    third, half = D // 3, Sk // 2

    def kernel_function(
        q_ref, k_ref, v_ref, o_ref, p_ref, r_ref, redo_ref, s_refs, l_refs
    ):
        step = pl.program_id(0)

        def put_probs(u, s, m):
            p = jnp.exp2(s - m)
            p_ref[u] = pltpu.bitcast(p.astype(bf16), u32)
            r_ref[u] = 1.0 / jnp.sum(_fold(p, 32), axis=0, keepdims=True)

        def body(do_scores, do_values):
            row_max, unsafe = {}, []

            def prepare_keys(h):
                l_ref = l_refs[h % _K_SLOTS]
                for j in range(0, half, _LANES):
                    k1a, k1b, k1c, k2a, k2b, k2c = (
                        k_ref[h, d : d + third, j0 : j0 + _LANES]
                        for j0 in (j, half + j)
                        for d in range(0, D, third)
                    )
                    b1, c1, b2, c2 = (x.astype(f32) for x in (k1b, k1c, k2b, k2c))
                    db, dc = b1 - b2, c2 - c1
                    db16, dc16 = db.astype(bf16), dc.astype(bf16)
                    n1 = _fold(jnp.abs(b1) + jnp.abs(c1))
                    n2 = _fold(jnp.abs(b2) + jnp.abs(c2))
                    e1 = _fold(jnp.abs(db - db16.astype(f32)))
                    e2 = _fold(jnp.abs(dc - dc16.astype(f32)))
                    t1, t2 = (
                        jnp.sum(e + 2.0**-20 * other - 2.0**-9 * own, 0, keepdims=True)
                        for e, own, other in ((e1, n1, n2), (e2, n2, n1))
                    )
                    bad = jnp.where((t1 <= 0) & (t2 <= 0), 0.0, 1.0)
                    unsafe.append(jnp.maximum(unsafe.pop(), bad) if unsafe else bad)
                    for n, pair in enumerate(((k2b, k1c), (k1a, db16), (k2a, dc16))):
                        r = (n * half + j) // 2
                        l_ref[r : r + _LANES // 2] = pltpu.bitcast(
                            jnp.concatenate(pair, 0).T, u32
                        )
                if h == _HEADS - 1:
                    redo_ref[0] = jnp.max(unsafe[0])

            def scores(u):
                h, t = divmod(u, tiles)
                cols = slice(t * _LANES, (t + 1) * _LANES)
                l_ref, s_ref = l_refs[h % _K_SLOTS], s_refs[u % _S_SLOTS]
                m = None
                for a, b in ((0, 3 * half // 4), (3 * half // 4, half)):
                    l5, l1, l2 = (
                        pltpu.bitcast(
                            l_ref[(n * half + a) // 2 : (n * half + b) // 2], bf16
                        )
                        for n in range(3)
                    )
                    f5 = _dot(l5, q_ref[h, third:, cols])
                    f1 = _dot(l1, q_ref[h, : 2 * third, cols])
                    qac = (q_ref[h, :third, cols], q_ref[h, 2 * third :, cols])
                    f2 = _dot(l2, jnp.concatenate(qac, 0))
                    s1, s2 = (f1 + f5) * log2_scale, (f2 + f5) * log2_scale
                    s_ref[a:b] = s1
                    s_ref[half + a : half + b] = s2
                    part = jnp.max(jnp.maximum(s1, s2).reshape(-1, 8, _LANES), axis=0)
                    m = part if m is None else jnp.maximum(m, part)
                row_max[u] = jnp.max(m, axis=0, keepdims=True)

            def probs(u):
                put_probs(u, s_refs[u % _S_SLOTS][...], row_max.pop(u))

            def values(u):
                h, t = divmod(u, tiles)
                o = _dot(v_ref[h], pltpu.bitcast(p_ref[u], bf16))
                o_ref[h, :, t * _LANES : (t + 1) * _LANES] = (o * r_ref[u]).astype(bf16)

            if do_values:
                values(0)
            if do_scores:
                prepare_keys(0)
                scores(0)
                scores(1)
            for u in range(2, units):
                if do_scores:
                    if u % tiles == 3 and u // tiles + 1 < _HEADS:
                        prepare_keys(u // tiles + 1)
                    scores(u)
                    probs(u - 2)
                if do_values:
                    values(u - 1)
            if do_scores:
                probs(units - 2)
            if do_values:
                values(units - 1)
            if do_scores:
                probs(units - 1)

        pl.when(step == 0)(lambda: body(True, False))
        pl.when((step > 0) & (step < n_blocks))(lambda: body(True, True))
        pl.when(step == n_blocks)(lambda: body(False, True))

        @pl.when((redo_ref[0] > 0) & (step < n_blocks))
        def _():
            def redo(h, carry):
                keys = k_ref[h].T
                for t in range(tiles):
                    s = _dot(keys, q_ref[h, :, t * _LANES : (t + 1) * _LANES])
                    s = s * log2_scale
                    put_probs(h * tiles + t, s, jnp.max(s, axis=0, keepdims=True))
                return carry

            jax.lax.fori_loop(0, _HEADS, redo, 0)

    def current(i):
        return jnp.minimum(i, n_blocks - 1), 0, 0

    def previous(i):
        return jnp.maximum(i - 1, 0), 0, 0

    qT, kT, vT = (
        jnp.swapaxes(x, 2, 3).reshape(B * H, D, x.shape[2]) for x in (q, k, v)
    )
    oT = pl.pallas_call(
        kernel_function,
        grid=(n_blocks + 1,),
        in_specs=[
            pl.BlockSpec((_HEADS, D, tiles * _LANES), current),
            pl.BlockSpec((_HEADS, D, Sk), current),
            pl.BlockSpec((_HEADS, D, Sk), previous),
        ],
        out_specs=pl.BlockSpec((_HEADS, D, tiles * _LANES), previous),
        out_shape=jax.ShapeDtypeStruct((B * H, D, Sq), q.dtype),
        scratch_shapes=[
            pltpu.VMEM((units, Sk // 2, _LANES), u32),
            pltpu.VMEM((units, 1, _LANES), f32),
            pltpu.SMEM((1,), f32),
            [pltpu.VMEM((Sk, _LANES), f32) for _ in range(_S_SLOTS)],
            [pltpu.VMEM((3 * half // 2, 2 * third), u32) for _ in range(_K_SLOTS)],
        ],
        compiler_params=pltpu.CompilerParams(
            dimension_semantics=("arbitrary",),
            vmem_limit_bytes=100 * 1024 * 1024,
        ),
    )(qT, kT, vT)
    return jnp.swapaxes(oT.reshape(B, H, D, Sq), 2, 3)
```

```python
import jax
import jax.numpy as jnp
import jax.experimental.pallas as pl
import jax.experimental.pallas.tpu as pltpu
import ml_dtypes
import numpy as np

_HEADS = 8
_LANES = 128
_S_SLOTS = 3


def _dot(a, b):
    return jnp.dot(a, b, preferred_element_type=jnp.float32)


def _fold(x, rows=8):
    return jnp.sum(x.reshape(-1, rows, x.shape[-1]), axis=0)


def _reciprocal(x):
    r = pl.reciprocal(x, approx=True)
    return r + r * (1.0 - x * r)


def _words(x):
    return pltpu.bitcast(x, jnp.uint32)


def _bf16(x):
    return pltpu.bitcast(x, jnp.bfloat16)


@jax.jit
def pallas_standalone__gqa_softmax__near_ridge_kernel(
    q: jax.Array,
    k: jax.Array,
    v: jax.Array,
):
    B, H, Sq, D = q.shape
    Sk = k.shape[2]
    assert k.shape == v.shape == (B, H, Sk, D)
    assert q.dtype == k.dtype == v.dtype == jnp.bfloat16
    f32, bf16, u32 = jnp.float32, jnp.bfloat16, jnp.uint32

    scale = float(np.asarray(D**-0.5, dtype=ml_dtypes.bfloat16))
    log2_scale = scale * float(np.log2(np.e))

    n_blocks = B * H // _HEADS
    tiles, rest = divmod(Sq, _LANES)
    units = _HEADS * tiles
    third, half = D // 3, Sk // 2
    rest_cols = slice(tiles * _LANES, (tiles + 1) * _LANES)
    assert D == 192 and Sk == 512 and n_blocks * _HEADS == B * H
    assert tiles >= 5 and rest > 0 and rest % 16 == 0

    def kernel_function(
        q_ref, k_ref, v_ref, o_ref,
        p_ref, r_ref, rest_p_ref, rest_r_ref, redo_ref,
        s_refs, keys_refs, diff_refs, rest_q_refs, rest_s_refs, rest_m_ref,
    ):
        step = pl.program_id(0)

        def query_pairs(h, cols):
            qac = (q_ref[h, :third, cols], q_ref[h, 2 * third :, cols])
            return (
                q_ref[h, third:, cols],
                q_ref[h, : 2 * third, cols],
                jnp.concatenate(qac, 0),
            )

        def put_probs(u, s_ref, m):
            even, odd = (
                jnp.exp2(s_ref[pl.ds(j, half, stride=2)] - m) for j in range(2)
            )
            p_ref[u] = pltpu.pack_elementwise([even, odd], packed_dtype=bf16)
            total = jnp.sum(_fold(even + odd, 32), axis=0, keepdims=True)
            r_ref[u] = _reciprocal(total)

        def put_rest_probs(h, s_ref):
            m = jnp.max(s_ref[...], axis=1, keepdims=True)
            rest_m_ref[h] = jnp.broadcast_to(m, (rest, _LANES))
            m = jnp.concatenate([rest_m_ref[h]] * (Sk // _LANES), 1)
            p = jnp.exp2(s_ref[...] - m)
            rest_p_ref[h] = _words(p.astype(bf16))
            a, b, c, d = (p[:, j : j + _LANES] for j in range(0, Sk, _LANES))
            total = jnp.sum((a + b) + (c + d), axis=1, keepdims=True)
            rest_r_ref[h] = jnp.broadcast_to(_reciprocal(total), (rest, _LANES))

        def body(do_scores, do_values):
            col_max, unsafe = {}, []

            def prepare_keys(h):
                for j in range(0, half, _LANES):
                    k1a, k1b, k1c, k2a, k2b, k2c = (
                        k_ref[h, d : d + third, j0 : j0 + _LANES]
                        for j0 in (j, half + j)
                        for d in range(0, D, third)
                    )
                    b1, c1, b2, c2 = (x.astype(f32) for x in (k1b, k1c, k2b, k2c))
                    db, dc = b1 - b2, c2 - c1
                    db16, dc16 = db.astype(bf16), dc.astype(bf16)
                    n1 = _fold(jnp.abs(b1) + jnp.abs(c1))
                    n2 = _fold(jnp.abs(b2) + jnp.abs(c2))
                    e1 = _fold(jnp.abs(db - db16.astype(f32)))
                    e2 = _fold(jnp.abs(dc - dc16.astype(f32)))
                    t1, t2 = (
                        jnp.sum(e + 2.0**-20 * other - 2.0**-9 * own, 0, keepdims=True)
                        for e, own, other in ((e1, n1, n2), (e2, n2, n1))
                    )
                    bad = jnp.where((t1 <= 0) & (t2 <= 0), 0.0, 1.0)
                    unsafe.append(jnp.maximum(unsafe.pop(), bad) if unsafe else bad)
                    diff_refs[h][0, :, j : j + _LANES] = _words(db16)
                    diff_refs[h][1, :, j : j + _LANES] = _words(dc16)
                    for n, pair in enumerate(((k2b, k1c), (k1a, db16), (k2a, dc16))):
                        keys_refs[h][n, j // 2 : (j + _LANES) // 2] = _words(
                            jnp.concatenate(pair, 0).T
                        )
                if h == _HEADS - 1:
                    redo_ref[0] = jnp.max(unsafe[0])
                for n, pair in enumerate(query_pairs(h, rest_cols)):
                    rest_q_refs[h][n] = _words(pair.T[:rest])

            def scores(u):
                h, t = divmod(u, tiles)
                s_ref, m = s_refs[u % _S_SLOTS], None
                for a, b in ((0, 3 * half // 4), (3 * half // 4, half)):
                    pairs = query_pairs(h, slice(t * _LANES, (t + 1) * _LANES))
                    f5, f1, f2 = (
                        _dot(_bf16(keys_refs[h][n, a // 2 : b // 2]), pairs[n])
                        for n in range(3)
                    )
                    s1, s2 = (f1 + f5) * log2_scale, (f2 + f5) * log2_scale
                    s_ref[a:b] = s1
                    s_ref[half + a : half + b] = s2
                    part = jnp.max(jnp.maximum(s1, s2).reshape(-1, 8, _LANES), axis=0)
                    m = part if m is None else jnp.maximum(m, part)
                col_max[u] = jnp.max(m, axis=0, keepdims=True)

            def probs(u):
                put_probs(u, s_refs[u % _S_SLOTS], col_max.pop(u))

            def values(u):
                h, t = divmod(u, tiles)
                o = _dot(v_ref[h], _bf16(p_ref[u])) * r_ref[u]
                o_ref[h, :, t * _LANES : (t + 1) * _LANES] = o.astype(bf16)

            def rest_scores(h):
                for j in range(0, half, _LANES):
                    one, two = slice(j, j + _LANES), slice(half + j, half + j + _LANES)
                    pairs = (
                        (k_ref[h, third : 2 * third, two], k_ref[h, 2 * third :, one]),
                        (k_ref[h, :third, one], _bf16(diff_refs[h][0, :, one])),
                        (k_ref[h, :third, two], _bf16(diff_refs[h][1, :, one])),
                    )
                    f5, f1, f2 = (
                        _dot(_bf16(rest_q_refs[h][n]), jnp.concatenate(pairs[n], 0))
                        for n in range(3)
                    )
                    rest_s_refs[h % 2][:, one] = (f1 + f5) * log2_scale
                    rest_s_refs[h % 2][:, two] = (f2 + f5) * log2_scale

            def rest_values(h):
                o = jax.lax.dot_general(
                    _bf16(rest_p_ref[h]), v_ref[h], (((1,), (1,)), ((), ())),
                    preferred_element_type=f32,
                )
                r = rest_r_ref[h]
                o = (o[:, :_LANES] * r, o[:, _LANES:] * r[:, : D - _LANES])
                o = jnp.concatenate(o, 1).astype(bf16)
                o = jnp.concatenate([o, jnp.zeros((_LANES - rest, D), bf16)], 0)
                o_ref[h, :, rest_cols] = o.T

            if do_values:
                values(0)
            if do_scores:
                prepare_keys(0)
                scores(0)
                scores(1)
            for u in range(2, units):
                h, t = divmod(u, tiles)
                if do_scores:
                    if t == 2 and h + 1 < _HEADS:
                        prepare_keys(h + 1)
                    scores(u)
                    probs(u - 2)
                if do_values:
                    values(u - 1)
                if do_values and (h % 2, t) == (0, 4):
                    rest_values(h)
                    rest_values(h + 1)
                if do_scores and (h % 2, t) == (1, 2):
                    rest_scores(h - 1)
                    rest_scores(h)
                if do_scores and (h % 2, t) == (1, 4):
                    put_rest_probs(h - 1, rest_s_refs[0])
                    put_rest_probs(h, rest_s_refs[1])
            if do_scores:
                probs(units - 2)
            if do_values:
                values(units - 1)
            if do_scores:
                probs(units - 1)

        pl.when(step == 0)(lambda: body(True, False))
        pl.when((step > 0) & (step < n_blocks))(lambda: body(True, True))
        pl.when(step == n_blocks)(lambda: body(False, True))

        @pl.when((redo_ref[0] > 0) & (step < n_blocks))
        def _():
            def redo(h, carry):
                keys = k_ref[h].T
                for t in range(tiles):
                    s = _dot(keys, q_ref[h, :, t * _LANES : (t + 1) * _LANES])
                    s = s * log2_scale
                    s_refs[0][...] = s
                    m = jnp.max(s, axis=0, keepdims=True)
                    put_probs(h * tiles + t, s_refs[0], m)
                s = _dot(q_ref[h, :, rest_cols].T[:rest], k_ref[h])
                rest_s_refs[0][...] = s * log2_scale
                put_rest_probs(h, rest_s_refs[0])
                return carry

            jax.lax.fori_loop(0, _HEADS, redo, 0)

    def current(i):
        return jnp.minimum(i, n_blocks - 1), 0, 0

    def previous(i):
        return jnp.maximum(i - 1, 0), 0, 0

    def per_head(shape, dtype, n=_HEADS):
        return [pltpu.VMEM(shape, dtype) for _ in range(n)]

    qT, kT, vT = (
        jnp.swapaxes(x, 2, 3).reshape(B * H, D, x.shape[2]) for x in (q, k, v)
    )
    oT = pl.pallas_call(
        kernel_function,
        grid=(n_blocks + 1,),
        in_specs=[
            pl.BlockSpec((_HEADS, D, rest_cols.stop), current),
            pl.BlockSpec((_HEADS, D, Sk), current),
            pl.BlockSpec((_HEADS, D, Sk), previous),
        ],
        out_specs=pl.BlockSpec((_HEADS, D, rest_cols.stop), previous),
        out_shape=jax.ShapeDtypeStruct((B * H, D, Sq), q.dtype),
        scratch_shapes=[
            pltpu.VMEM((units, half, _LANES), u32),
            pltpu.VMEM((units, 1, _LANES), f32),
            pltpu.VMEM((_HEADS, rest // 2, Sk), u32),
            pltpu.VMEM((_HEADS, rest, _LANES), f32),
            pltpu.SMEM((1,), f32),
            per_head((Sk, _LANES), f32, _S_SLOTS),
            per_head((3, half // 2, 2 * third), u32),
            per_head((2, third // 2, half), u32),
            per_head((3, rest // 2, 2 * third), u32),
            per_head((rest, Sk), f32, 2),
            pltpu.VMEM((_HEADS, rest, _LANES), f32),
        ],
        compiler_params=pltpu.CompilerParams(
            dimension_semantics=("arbitrary",),
            vmem_limit_bytes=100 * 1024 * 1024,
        ),
    )(qT, kT, vT)
    return jnp.swapaxes(oT.reshape(B, H, D, Sq), 2, 3)
```

```python
import jax
import jax.numpy as jnp
import jax.experimental.pallas as pl
import jax.experimental.pallas.tpu as pltpu
import ml_dtypes
import numpy as np

_HEADS = 8
_LANES = 128
_S_SLOTS = 4


def _dot(a, b):
    return jnp.dot(a, b, preferred_element_type=jnp.float32)


def _dot_t(a, b):
    dims = (((1,), (1,)), ((), ()))
    return jax.lax.dot_general(a, b, dims, preferred_element_type=jnp.float32)


def _pad_rows(x):
    zeros = jnp.zeros((_LANES - x.shape[0], x.shape[1]), x.dtype)
    return jnp.concatenate([x, zeros], 0)


def _fold(x, rows=8):
    return jnp.sum(x.reshape(-1, rows, x.shape[-1]), axis=0)


def _reciprocal(x):
    r = pl.reciprocal(x, approx=True)
    return r + r * (1.0 - x * r)


def _words(x):
    return pltpu.bitcast(x, jnp.uint32)


def _bf16(x):
    return pltpu.bitcast(x, jnp.bfloat16)


@jax.jit
def pallas_standalone__gqa_softmax__near_ridge_kernel(
    q: jax.Array,
    k: jax.Array,
    v: jax.Array,
):
    B, H, Sq, D = q.shape
    Sk = k.shape[2]
    assert k.shape == v.shape == (B, H, Sk, D)
    assert q.dtype == k.dtype == v.dtype == jnp.bfloat16
    f32, bf16, u32 = jnp.float32, jnp.bfloat16, jnp.uint32

    scale = float(np.asarray(D**-0.5, dtype=ml_dtypes.bfloat16))
    log2_scale = scale * float(np.log2(np.e))

    n_blocks = B * H // _HEADS
    tiles, rest = divmod(Sq, _LANES)
    units = _HEADS * tiles
    third, half = D // 3, Sk // 2
    rest_cols = slice(tiles * _LANES, (tiles + 1) * _LANES)
    assert D == 192 and Sk == 512 and n_blocks * _HEADS == B * H
    assert tiles >= 5 and rest > 0 and rest % 16 == 0

    def kernel_function(
        q_ref, k_ref, v_ref, o_ref,
        p_ref, r_ref, rest_p_ref, rest_r_ref, redo_ref,
        s_refs, keys_refs, diff_refs, rest_q_refs, rest_s_refs, rest_m_ref,
    ):
        step = pl.program_id(0)

        def query_pairs(h, cols):
            qac = (q_ref[h, :third, cols], q_ref[h, 2 * third :, cols])
            return (
                q_ref[h, third:, cols],
                q_ref[h, : 2 * third, cols],
                jnp.concatenate(qac, 0),
            )

        def put_probs(u, s_ref, m):
            even, odd = (
                jnp.exp2(s_ref[pl.ds(j, half, stride=2)] - m) for j in range(2)
            )
            p_ref[u] = pltpu.pack_elementwise([even, odd], packed_dtype=bf16)
            total = jnp.sum(_fold(even + odd, 32), axis=0, keepdims=True)
            r_ref[u] = _reciprocal(total)

        def put_rest_probs(h, s_ref):
            m = jnp.max(s_ref[...], axis=1, keepdims=True)
            rest_m_ref[h] = jnp.broadcast_to(m, (rest, _LANES))
            m = jnp.concatenate([rest_m_ref[h]] * (Sk // _LANES), 1)
            p = jnp.exp2(s_ref[...] - m)
            rest_p_ref[h] = _words(p.astype(bf16))
            a, b, c, d = (p[:, j : j + _LANES] for j in range(0, Sk, _LANES))
            total = jnp.sum((a + b) + (c + d), axis=1, keepdims=True)
            rest_r_ref[h] = jnp.broadcast_to(_reciprocal(total), (rest, _LANES))

        def body(do_scores, do_values):
            col_max, unsafe = {}, []

            def prepare_keys(h):
                for j in range(0, half, _LANES):
                    k1a, k1b, k1c, k2a, k2b, k2c = (
                        k_ref[h, d : d + third, j0 : j0 + _LANES]
                        for j0 in (j, half + j)
                        for d in range(0, D, third)
                    )
                    b1, c1, b2, c2 = (x.astype(f32) for x in (k1b, k1c, k2b, k2c))
                    db, dc = b1 - b2, c2 - c1
                    db16, dc16 = db.astype(bf16), dc.astype(bf16)
                    n1 = _fold(jnp.abs(b1) + jnp.abs(c1))
                    n2 = _fold(jnp.abs(b2) + jnp.abs(c2))
                    e1 = _fold(jnp.abs(db - db16.astype(f32)))
                    e2 = _fold(jnp.abs(dc - dc16.astype(f32)))
                    t1, t2 = (
                        jnp.sum(e + 2.0**-20 * other - 2.0**-9 * own, 0, keepdims=True)
                        for e, own, other in ((e1, n1, n2), (e2, n2, n1))
                    )
                    bad = jnp.where((t1 <= 0) & (t2 <= 0), 0.0, 1.0)
                    unsafe.append(jnp.maximum(unsafe.pop(), bad) if unsafe else bad)
                    diff_refs[h][0, :, j : j + _LANES] = _words(db16)
                    diff_refs[h][1, :, j : j + _LANES] = _words(dc16)
                    for n, pair in enumerate(((k2b, k1c), (k1a, db16), (k2a, dc16))):
                        keys_refs[h][n, j // 2 : (j + _LANES) // 2] = _words(
                            jnp.concatenate(pair, 0).T
                        )
                if h == _HEADS - 1:
                    redo_ref[0] = jnp.max(unsafe[0])
                for n, pair in enumerate(query_pairs(h, rest_cols)):
                    rest_q_refs[h][n] = _words(pair.T[:rest])

            def scores(u):
                h, t = divmod(u, tiles)
                s_ref, m = s_refs[u % _S_SLOTS], None
                for a, b in ((0, 3 * half // 4), (3 * half // 4, half)):
                    pairs = query_pairs(h, slice(t * _LANES, (t + 1) * _LANES))
                    f5, f1, f2 = (
                        _dot(_bf16(keys_refs[h][n, a // 2 : b // 2]), pairs[n])
                        for n in range(3)
                    )
                    s1, s2 = (f1 + f5) * log2_scale, (f2 + f5) * log2_scale
                    s_ref[a:b] = s1
                    s_ref[half + a : half + b] = s2
                    part = jnp.max(jnp.maximum(s1, s2).reshape(-1, 8, _LANES), axis=0)
                    m = part if m is None else jnp.maximum(m, part)
                col_max[u] = jnp.max(m, axis=0, keepdims=True)

            def probs(u):
                put_probs(u, s_refs[u % _S_SLOTS], col_max.pop(u))

            def values(u):
                h, t = divmod(u, tiles)
                o = _dot(v_ref[h], _bf16(p_ref[u])) * r_ref[u]
                o_ref[h, :, t * _LANES : (t + 1) * _LANES] = o.astype(bf16)

            def rest_scores(h):
                for j in range(0, half, _LANES):
                    one, two = slice(j, j + _LANES), slice(half + j, half + j + _LANES)
                    pairs = (
                        (k_ref[h, third : 2 * third, two], k_ref[h, 2 * third :, one]),
                        (k_ref[h, :third, one], _bf16(diff_refs[h][0, :, one])),
                        (k_ref[h, :third, two], _bf16(diff_refs[h][1, :, one])),
                    )
                    f5, f1, f2 = (
                        _dot(_bf16(rest_q_refs[h][n]), jnp.concatenate(pairs[n], 0))
                        for n in range(3)
                    )
                    rest_s_refs[h % 2][:, one] = (f1 + f5) * log2_scale
                    rest_s_refs[h % 2][:, two] = (f2 + f5) * log2_scale

            def rest_values_low(h):
                o = _dot_t(_bf16(rest_p_ref[h]), v_ref[h, :_LANES]) * rest_r_ref[h]
                o_ref[h, :_LANES, rest_cols] = _pad_rows(o.astype(bf16)).T

            def rest_values_high(h):
                o = _dot_t(v_ref[h, _LANES:], _pad_rows(_bf16(rest_p_ref[h])))
                o = o * _pad_rows(rest_r_ref[h]).T[:1]
                o_ref[h, _LANES:, rest_cols] = o.astype(bf16)

            if do_values:
                values(0)
            if do_scores:
                prepare_keys(0)
            for u in range(units):
                h, t = divmod(u, tiles)
                pair = (h - h % 2, h - h % 2 + 1)
                if do_scores:
                    if t == 2 and h + 1 < _HEADS:
                        prepare_keys(h + 1)
                    scores(u)
                    if u >= 3:
                        probs(u - 3)
                if do_values and u >= 3:
                    values(u - 2)
                for g in pair:
                    if do_values and (h % 2, t) == (0, 4):
                        rest_values_low(g)
                    if do_values and (h % 2, t) == (1, 0):
                        rest_values_high(g)
                    if do_scores and (h % 2, t) == (1, 2):
                        rest_scores(g)
                    if do_scores and (h % 2, t) == (1, 4):
                        put_rest_probs(g, rest_s_refs[g % 2])
            for u in range(units - 3, units):
                if do_values and u >= units - 2:
                    values(u)
                if do_scores:
                    probs(u)

        pl.when(step == 0)(lambda: body(True, False))
        pl.when((step > 0) & (step < n_blocks))(lambda: body(True, True))
        pl.when(step == n_blocks)(lambda: body(False, True))

        @pl.when((redo_ref[0] > 0) & (step < n_blocks))
        def _():
            def redo(h, carry):
                keys = k_ref[h].T
                for t in range(tiles):
                    s = _dot(keys, q_ref[h, :, t * _LANES : (t + 1) * _LANES])
                    s = s * log2_scale
                    s_refs[0][...] = s
                    m = jnp.max(s, axis=0, keepdims=True)
                    put_probs(h * tiles + t, s_refs[0], m)
                s = _dot(q_ref[h, :, rest_cols].T[:rest], k_ref[h])
                rest_s_refs[0][...] = s * log2_scale
                put_rest_probs(h, rest_s_refs[0])
                return carry

            jax.lax.fori_loop(0, _HEADS, redo, 0)

    def current(i):
        return jnp.minimum(i, n_blocks - 1), 0, 0

    def previous(i):
        return jnp.maximum(i - 1, 0), 0, 0

    def per_head(shape, dtype, n=_HEADS):
        return [pltpu.VMEM(shape, dtype) for _ in range(n)]

    qT, kT, vT = (
        jnp.swapaxes(x, 2, 3).reshape(B * H, D, x.shape[2]) for x in (q, k, v)
    )
    oT = pl.pallas_call(
        kernel_function,
        grid=(n_blocks + 1,),
        in_specs=[
            pl.BlockSpec((_HEADS, D, rest_cols.stop), current),
            pl.BlockSpec((_HEADS, D, Sk), current),
            pl.BlockSpec((_HEADS, D, Sk), previous),
        ],
        out_specs=pl.BlockSpec((_HEADS, D, rest_cols.stop), previous),
        out_shape=jax.ShapeDtypeStruct((B * H, D, Sq), q.dtype),
        scratch_shapes=[
            pltpu.VMEM((units, half, _LANES), u32),
            pltpu.VMEM((units, 1, _LANES), f32),
            pltpu.VMEM((_HEADS, rest // 2, Sk), u32),
            pltpu.VMEM((_HEADS, rest, _LANES), f32),
            pltpu.SMEM((1,), f32),
            per_head((Sk, _LANES), f32, _S_SLOTS),
            per_head((3, half // 2, 2 * third), u32),
            per_head((2, third // 2, half), u32),
            per_head((3, rest // 2, 2 * third), u32),
            per_head((rest, Sk), f32, 2),
            pltpu.VMEM((_HEADS, rest, _LANES), f32),
        ],
        compiler_params=pltpu.CompilerParams(
            dimension_semantics=("arbitrary",),
            vmem_limit_bytes=100 * 1024 * 1024,
            disable_bounds_checks=True,
        ),
    )(qT, kT, vT)
    return jnp.swapaxes(oT.reshape(B, H, D, Sq), 2, 3)
```

```python
import jax
import jax.numpy as jnp
import jax.experimental.pallas as pl
import jax.experimental.pallas.tpu as pltpu
import ml_dtypes
import numpy as np

_HEADS = 8
_LANES = 128
_S_SLOTS = 4


def _dot(a, b):
    return jnp.dot(a, b, preferred_element_type=jnp.float32)


def _dot_t(a, b):
    dims = (((1,), (1,)), ((), ()))
    return jax.lax.dot_general(a, b, dims, preferred_element_type=jnp.float32)


def _pad_rows(x):
    zeros = jnp.zeros((_LANES - x.shape[0], x.shape[1]), x.dtype)
    return jnp.concatenate([x, zeros], 0)


def _fold(x, rows=8):
    return jnp.sum(x.reshape(-1, rows, x.shape[-1]), axis=0)


def _reciprocal(x):
    r = pl.reciprocal(x, approx=True)
    return r + r * (1.0 - x * r)


def _words(x):
    return pltpu.bitcast(x, jnp.uint32)


def _bf16(x):
    return pltpu.bitcast(x, jnp.bfloat16)


@jax.jit
def pallas_standalone__gqa_softmax__near_ridge_kernel(
    q: jax.Array,
    k: jax.Array,
    v: jax.Array,
):
    B, H, Sq, D = q.shape
    Sk = k.shape[2]
    assert k.shape == v.shape == (B, H, Sk, D)
    assert q.dtype == k.dtype == v.dtype == jnp.bfloat16
    f32, bf16, u32 = jnp.float32, jnp.bfloat16, jnp.uint32

    scale = float(np.asarray(D**-0.5, dtype=ml_dtypes.bfloat16))
    log2_scale = scale * float(np.log2(np.e))

    n_blocks = B * H // _HEADS
    tiles, rest = divmod(Sq, _LANES)
    units = _HEADS * tiles
    third, half = D // 3, Sk // 2
    rest_cols = slice(tiles * _LANES, (tiles + 1) * _LANES)
    assert D == 192 and Sk == 512 and n_blocks * _HEADS == B * H
    assert tiles >= 5 and rest > 0 and rest % 16 == 0

    def kernel_function(
        q_ref, k_ref, v_ref, o_ref,
        p_ref, r_ref, rest_p_ref, rest_r_ref, redo_ref,
        s_refs, keys_refs, diff_refs, rest_q_refs, rest_s_refs, rest_m_ref,
    ):
        step = pl.program_id(0)

        def query_pairs(h, cols):
            qac = (q_ref[h, :third, cols], q_ref[h, 2 * third :, cols])
            return (
                q_ref[h, third:, cols],
                q_ref[h, : 2 * third, cols],
                jnp.concatenate(qac, 0),
            )

        def put_probs(u, s, m):
            p = jnp.exp2(s - m)
            p_ref[u] = p.astype(bf16)
            r_ref[u] = _reciprocal(jnp.sum(_fold(p, 64), axis=0, keepdims=True))

        def put_rest_probs(h, s_ref):
            m = jnp.max(s_ref[...], axis=1, keepdims=True)
            rest_m_ref[h] = jnp.broadcast_to(m, (rest, _LANES))
            m = jnp.concatenate([rest_m_ref[h]] * (Sk // _LANES), 1)
            p = jnp.exp2(s_ref[...] - m)
            rest_p_ref[h] = _words(p.astype(bf16))
            a, b, c, d = (p[:, j : j + _LANES] for j in range(0, Sk, _LANES))
            total = jnp.sum((a + b) + (c + d), axis=1, keepdims=True)
            rest_r_ref[h] = jnp.broadcast_to(_reciprocal(total), (rest, _LANES))

        def body(do_scores, do_values):
            col_max, unsafe = {}, []

            def prepare_keys(h):
                for j in range(0, half, _LANES):
                    k1a, k1b, k1c, k2a, k2b, k2c = (
                        k_ref[h, d : d + third, j0 : j0 + _LANES]
                        for j0 in (j, half + j)
                        for d in range(0, D, third)
                    )
                    b1, c1, b2, c2 = (x.astype(f32) for x in (k1b, k1c, k2b, k2c))
                    db, dc = b1 - b2, c2 - c1
                    db16, dc16 = db.astype(bf16), dc.astype(bf16)
                    n1 = _fold(jnp.abs(b1) + jnp.abs(c1))
                    n2 = _fold(jnp.abs(b2) + jnp.abs(c2))
                    e1 = _fold(jnp.abs(db - db16.astype(f32)))
                    e2 = _fold(jnp.abs(dc - dc16.astype(f32)))
                    t1, t2 = (
                        jnp.sum(e + 2.0**-20 * other - 2.0**-9 * own, 0, keepdims=True)
                        for e, own, other in ((e1, n1, n2), (e2, n2, n1))
                    )
                    bad = jnp.where((t1 <= 0) & (t2 <= 0), 0.0, 1.0)
                    unsafe.append(jnp.maximum(unsafe.pop(), bad) if unsafe else bad)
                    diff_refs[h][0, :, j : j + _LANES] = _words(db16)
                    diff_refs[h][1, :, j : j + _LANES] = _words(dc16)
                    for n, pair in enumerate(((k2b, k1c), (k1a, db16), (k2a, dc16))):
                        keys_refs[h][n, j // 2 : (j + _LANES) // 2] = _words(
                            jnp.concatenate(pair, 0).T
                        )
                if h == _HEADS - 1:
                    redo_ref[0] = jnp.max(unsafe[0])
                for n, pair in enumerate(query_pairs(h, rest_cols)):
                    rest_q_refs[h][n] = _words(pair.T[:rest])

            def scores(u):
                h, t = divmod(u, tiles)
                s_ref, m = s_refs[u % _S_SLOTS], None
                for a, b in ((0, 3 * half // 4), (3 * half // 4, half)):
                    pairs = query_pairs(h, slice(t * _LANES, (t + 1) * _LANES))
                    f5, f1, f2 = (
                        _dot(_bf16(keys_refs[h][n, a // 2 : b // 2]), pairs[n])
                        for n in range(3)
                    )
                    s1, s2 = (f1 + f5) * log2_scale, (f2 + f5) * log2_scale
                    s_ref[a:b] = s1
                    s_ref[half + a : half + b] = s2
                    part = jnp.max(jnp.maximum(s1, s2).reshape(-1, 8, _LANES), axis=0)
                    m = part if m is None else jnp.maximum(m, part)
                col_max[u] = jnp.max(m, axis=0, keepdims=True)

            def probs(u):
                put_probs(u, s_refs[u % _S_SLOTS][...], col_max.pop(u))

            def values(u):
                h, t = divmod(u, tiles)
                o = _dot(v_ref[h], p_ref[u]) * r_ref[u]
                o_ref[h, :, t * _LANES : (t + 1) * _LANES] = o.astype(bf16)

            def rest_scores(h):
                for j in range(0, half, _LANES):
                    one, two = slice(j, j + _LANES), slice(half + j, half + j + _LANES)
                    pairs = (
                        (k_ref[h, third : 2 * third, two], k_ref[h, 2 * third :, one]),
                        (k_ref[h, :third, one], _bf16(diff_refs[h][0, :, one])),
                        (k_ref[h, :third, two], _bf16(diff_refs[h][1, :, one])),
                    )
                    f5, f1, f2 = (
                        _dot(_bf16(rest_q_refs[h][n]), jnp.concatenate(pairs[n], 0))
                        for n in range(3)
                    )
                    rest_s_refs[h % 2][:, one] = (f1 + f5) * log2_scale
                    rest_s_refs[h % 2][:, two] = (f2 + f5) * log2_scale

            def rest_values_low(h):
                o = _dot_t(_bf16(rest_p_ref[h]), v_ref[h, :_LANES]) * rest_r_ref[h]
                o_ref[h, :_LANES, rest_cols] = _pad_rows(o.astype(bf16)).T

            def rest_values_high(h):
                o = _dot_t(v_ref[h, _LANES:], _pad_rows(_bf16(rest_p_ref[h])))
                o = o * _pad_rows(rest_r_ref[h]).T[:1]
                o_ref[h, _LANES:, rest_cols] = o.astype(bf16)

            if do_values:
                values(0)
            if do_scores:
                prepare_keys(0)
            for u in range(units):
                h, t = divmod(u, tiles)
                pair = (h - h % 2, h - h % 2 + 1)
                if do_scores:
                    if t == 2 and h + 1 < _HEADS:
                        prepare_keys(h + 1)
                    scores(u)
                    if u >= 3:
                        probs(u - 3)
                if do_values and u >= 3:
                    values(u - 2)
                for g in pair:
                    if do_values and (h % 2, t) == (0, 4):
                        rest_values_low(g)
                    if do_values and (h % 2, t) == (1, 0):
                        rest_values_high(g)
                    if do_scores and (h % 2, t) == (1, 2):
                        rest_scores(g)
                    if do_scores and (h % 2, t) == (1, 4):
                        put_rest_probs(g, rest_s_refs[g % 2])
            for u in range(units - 3, units):
                if do_values and u >= units - 2:
                    values(u)
                if do_scores:
                    probs(u)

        pl.when(step == 0)(lambda: body(True, False))
        pl.when((step > 0) & (step < n_blocks))(lambda: body(True, True))
        pl.when(step == n_blocks)(lambda: body(False, True))

        @pl.when((redo_ref[0] > 0) & (step < n_blocks))
        def _():
            def redo(h, carry):
                keys = k_ref[h].T
                for t in range(tiles):
                    s = _dot(keys, q_ref[h, :, t * _LANES : (t + 1) * _LANES])
                    s = s * log2_scale
                    put_probs(h * tiles + t, s, jnp.max(s, axis=0, keepdims=True))
                s = _dot(q_ref[h, :, rest_cols].T[:rest], k_ref[h])
                rest_s_refs[0][...] = s * log2_scale
                put_rest_probs(h, rest_s_refs[0])
                return carry

            jax.lax.fori_loop(0, _HEADS, redo, 0)

    def current(i):
        return jnp.minimum(i, n_blocks - 1), 0, 0

    def previous(i):
        return jnp.maximum(i - 1, 0), 0, 0

    def per_head(shape, dtype, n=_HEADS):
        return [pltpu.VMEM(shape, dtype) for _ in range(n)]

    qT, kT, vT = (
        jnp.swapaxes(x, 2, 3).reshape(B * H, D, x.shape[2]) for x in (q, k, v)
    )
    oT = pl.pallas_call(
        kernel_function,
        grid=(n_blocks + 1,),
        in_specs=[
            pl.BlockSpec((_HEADS, D, rest_cols.stop), current),
            pl.BlockSpec((_HEADS, D, Sk), current),
            pl.BlockSpec((_HEADS, D, Sk), previous),
        ],
        out_specs=pl.BlockSpec((_HEADS, D, rest_cols.stop), previous),
        out_shape=jax.ShapeDtypeStruct((B * H, D, Sq), q.dtype),
        scratch_shapes=[
            pltpu.VMEM((units, Sk, _LANES), bf16),
            pltpu.VMEM((units, 1, _LANES), f32),
            pltpu.VMEM((_HEADS, rest // 2, Sk), u32),
            pltpu.VMEM((_HEADS, rest, _LANES), f32),
            pltpu.SMEM((1,), f32),
            per_head((Sk, _LANES), f32, _S_SLOTS),
            per_head((3, half // 2, 2 * third), u32),
            per_head((2, third // 2, half), u32),
            per_head((3, rest // 2, 2 * third), u32),
            per_head((rest, Sk), f32, 2),
            pltpu.VMEM((_HEADS, rest, _LANES), f32),
        ],
        compiler_params=pltpu.CompilerParams(
            dimension_semantics=("arbitrary",),
            vmem_limit_bytes=100 * 1024 * 1024,
            disable_bounds_checks=True,
        ),
    )(qT, kT, vT)
    return jnp.swapaxes(oT.reshape(B, H, D, Sq), 2, 3)
```

```python
import jax
import jax.numpy as jnp
import jax.experimental.pallas as pl
import jax.experimental.pallas.tpu as pltpu
import ml_dtypes
import numpy as np

_HEADS = 8
_LANES = 128
_S_SLOTS = 4


def _dot(a, b):
    return jnp.dot(a, b, preferred_element_type=jnp.float32)


def _dot_t(a, b):
    dims = (((1,), (1,)), ((), ()))
    return jax.lax.dot_general(a, b, dims, preferred_element_type=jnp.float32)


def _pad_rows(x):
    zeros = jnp.zeros((_LANES - x.shape[0], x.shape[1]), x.dtype)
    return jnp.concatenate([x, zeros], 0)


def _fold(x, rows=8):
    return jnp.sum(x.reshape(-1, rows, x.shape[-1]), axis=0)


def _reciprocal(x):
    r = pl.reciprocal(x, approx=True)
    return r + r * (1.0 - x * r)


def _words(x):
    return pltpu.bitcast(x, jnp.uint32)


def _bf16(x):
    return pltpu.bitcast(x, jnp.bfloat16)


@jax.jit
def pallas_standalone__gqa_softmax__near_ridge_kernel(
    q: jax.Array,
    k: jax.Array,
    v: jax.Array,
):
    B, H, Sq, D = q.shape
    Sk = k.shape[2]
    assert k.shape == v.shape == (B, H, Sk, D)
    assert q.dtype == k.dtype == v.dtype == jnp.bfloat16
    f32, bf16, u32 = jnp.float32, jnp.bfloat16, jnp.uint32

    scale = float(np.asarray(D**-0.5, dtype=ml_dtypes.bfloat16))
    log2_scale = scale * float(np.log2(np.e))

    n_blocks = B * H // _HEADS
    tiles, rest = divmod(Sq, _LANES)
    units = _HEADS * tiles
    third, half = D // 3, Sk // 2
    rest_cols = slice(tiles * _LANES, (tiles + 1) * _LANES)
    assert D == 192 and Sk == 512 and n_blocks * _HEADS == B * H
    assert tiles >= 6 and rest > 0 and rest % 16 == 0

    def kernel_function(
        q_ref, k_ref, v_ref, o_ref,
        p_ref, r_ref, rest_p_ref, rest_r_ref, redo_ref,
        s_refs, keys_refs, diff_refs, rest_q_refs, rest_s_refs, rest_m_ref,
    ):
        step = pl.program_id(0)

        def query_pairs(h, cols):
            qac = (q_ref[h, :third, cols], q_ref[h, 2 * third :, cols])
            return (
                q_ref[h, third:, cols],
                q_ref[h, : 2 * third, cols],
                jnp.concatenate(qac, 0),
            )

        def put_probs(u, s, m):
            p = jnp.exp2(s - m)
            p_ref[u] = p.astype(bf16)
            r_ref[u] = _reciprocal(jnp.sum(_fold(p, 64), axis=0, keepdims=True))

        def put_rest_probs(h, s_ref):
            m = jnp.max(s_ref[...], axis=1, keepdims=True)
            rest_m_ref[h] = jnp.broadcast_to(m, (rest, _LANES))
            m = jnp.concatenate([rest_m_ref[h]] * (Sk // _LANES), 1)
            p = jnp.exp2(s_ref[...] - m)
            rest_p_ref[h] = p.astype(bf16)
            a, b, c, d = (p[:, j : j + _LANES] for j in range(0, Sk, _LANES))
            total = jnp.sum((a + b) + (c + d), axis=1, keepdims=True)
            rest_r_ref[h] = jnp.broadcast_to(_reciprocal(total), (rest, _LANES))

        def body(do_scores, do_values):
            col_max, unsafe = {}, []

            def prepare_keys(h):
                for j in range(0, half, _LANES):
                    k1a, k1b, k1c, k2a, k2b, k2c = (
                        k_ref[h, d : d + third, j0 : j0 + _LANES]
                        for j0 in (j, half + j)
                        for d in range(0, D, third)
                    )
                    b1, c1, b2, c2 = (x.astype(f32) for x in (k1b, k1c, k2b, k2c))
                    db, dc = b1 - b2, c2 - c1
                    db16, dc16 = db.astype(bf16), dc.astype(bf16)
                    n1 = _fold(jnp.abs(b1) + jnp.abs(c1))
                    n2 = _fold(jnp.abs(b2) + jnp.abs(c2))
                    e1 = _fold(jnp.abs(db - db16.astype(f32)))
                    e2 = _fold(jnp.abs(dc - dc16.astype(f32)))
                    t1, t2 = (
                        jnp.sum(e + 2.0**-20 * other - 2.0**-9 * own, 0, keepdims=True)
                        for e, own, other in ((e1, n1, n2), (e2, n2, n1))
                    )
                    bad = jnp.where((t1 <= 0) & (t2 <= 0), 0.0, 1.0)
                    unsafe.append(jnp.maximum(unsafe.pop(), bad) if unsafe else bad)
                    diff_refs[h][0, :, j : j + _LANES] = _words(db16)
                    diff_refs[h][1, :, j : j + _LANES] = _words(dc16)
                    for n, pair in enumerate(((k2b, k1c), (k1a, db16), (k2a, dc16))):
                        keys_refs[h][n, j // 2 : (j + _LANES) // 2] = _words(
                            jnp.concatenate(pair, 0).T
                        )
                if h == _HEADS - 1:
                    redo_ref[0] = jnp.max(unsafe[0])
                for n, pair in enumerate(query_pairs(h, rest_cols)):
                    rest_q_refs[h][n] = _words(pair.T[:rest])

            def scores(u):
                h, t = divmod(u, tiles)
                s_ref, m = s_refs[u % _S_SLOTS], None
                for a, b in ((0, 3 * half // 4), (3 * half // 4, half)):
                    pairs = query_pairs(h, slice(t * _LANES, (t + 1) * _LANES))
                    f5, f1, f2 = (
                        _dot(_bf16(keys_refs[h][n, a // 2 : b // 2]), pairs[n])
                        for n in range(3)
                    )
                    s1, s2 = (f1 + f5) * log2_scale, (f2 + f5) * log2_scale
                    s_ref[a:b] = s1
                    s_ref[half + a : half + b] = s2
                    part = jnp.max(jnp.maximum(s1, s2).reshape(-1, 8, _LANES), axis=0)
                    m = part if m is None else jnp.maximum(m, part)
                col_max[u] = jnp.max(m, axis=0, keepdims=True)

            def probs(u):
                put_probs(u, s_refs[u % _S_SLOTS][...], col_max.pop(u))

            def values(u):
                h, t = divmod(u, tiles)
                o = _dot(v_ref[h], p_ref[u]) * r_ref[u]
                o_ref[h, :, t * _LANES : (t + 1) * _LANES] = o.astype(bf16)

            def rest_scores(h):
                for j in range(0, half, _LANES):
                    one, two = slice(j, j + _LANES), slice(half + j, half + j + _LANES)
                    pairs = (
                        (k_ref[h, third : 2 * third, two], k_ref[h, 2 * third :, one]),
                        (k_ref[h, :third, one], _bf16(diff_refs[h][0, :, one])),
                        (k_ref[h, :third, two], _bf16(diff_refs[h][1, :, one])),
                    )
                    f5, f1, f2 = (
                        _dot(_bf16(rest_q_refs[h][n]), jnp.concatenate(pairs[n], 0))
                        for n in range(3)
                    )
                    rest_s_refs[h % 2][:, one] = (f1 + f5) * log2_scale
                    rest_s_refs[h % 2][:, two] = (f2 + f5) * log2_scale

            def rest_values_low(h):
                o = _dot_t(rest_p_ref[h], v_ref[h, :_LANES]) * rest_r_ref[h]
                o_ref[h, :_LANES, rest_cols] = _pad_rows(o.astype(bf16)).T

            def rest_values_high(h):
                o = _dot_t(v_ref[h, _LANES:], _pad_rows(rest_p_ref[h]))
                o = o * _pad_rows(rest_r_ref[h]).T[:1]
                o_ref[h, _LANES:, rest_cols] = o.astype(bf16)

            if do_values:
                values(0)
            if do_scores:
                prepare_keys(0)
            for u in range(units):
                h, t = divmod(u, tiles)
                pair = (h - h % 2, h - h % 2 + 1)
                if do_scores:
                    if t == 2 and h + 1 < _HEADS:
                        prepare_keys(h + 1)
                    scores(u)
                    if u >= 3:
                        probs(u - 3)
                if do_values and u >= 3:
                    values(u - 2)
                for g in pair:
                    if do_values and (h % 2, t) == (0, 3):
                        rest_values_low(g)
                    if do_values and (h % 2, t) == (0, 5):
                        rest_values_high(g)
                    if do_scores and (h % 2, t) == (1, 2):
                        rest_scores(g)
                    if do_scores and (h % 2, t) == (1, 4):
                        put_rest_probs(g, rest_s_refs[g % 2])
            for u in range(units - 3, units):
                if do_values and u >= units - 2:
                    values(u)
                if do_scores:
                    probs(u)

        pl.when(step == 0)(lambda: body(True, False))
        pl.when((step > 0) & (step < n_blocks))(lambda: body(True, True))
        pl.when(step == n_blocks)(lambda: body(False, True))

        @pl.when((redo_ref[0] > 0) & (step < n_blocks))
        def _():
            def redo(h, carry):
                keys = k_ref[h].T
                for t in range(tiles):
                    s = _dot(keys, q_ref[h, :, t * _LANES : (t + 1) * _LANES])
                    s = s * log2_scale
                    put_probs(h * tiles + t, s, jnp.max(s, axis=0, keepdims=True))
                s = _dot(q_ref[h, :, rest_cols].T[:rest], k_ref[h])
                rest_s_refs[0][...] = s * log2_scale
                put_rest_probs(h, rest_s_refs[0])
                return carry

            jax.lax.fori_loop(0, _HEADS, redo, 0)

    def current(i):
        return jnp.minimum(i, n_blocks - 1), 0, 0

    def previous(i):
        return jnp.maximum(i - 1, 0), 0, 0

    def per_head(shape, dtype, n=_HEADS):
        return [pltpu.VMEM(shape, dtype) for _ in range(n)]

    qT, kT, vT = (
        jnp.swapaxes(x, 2, 3).reshape(B * H, D, x.shape[2]) for x in (q, k, v)
    )
    oT = pl.pallas_call(
        kernel_function,
        grid=(n_blocks + 1,),
        in_specs=[
            pl.BlockSpec((_HEADS, D, rest_cols.stop), current),
            pl.BlockSpec((_HEADS, D, Sk), current),
            pl.BlockSpec((_HEADS, D, Sk), previous),
        ],
        out_specs=pl.BlockSpec((_HEADS, D, rest_cols.stop), previous),
        out_shape=jax.ShapeDtypeStruct((B * H, D, Sq), q.dtype),
        scratch_shapes=[
            pltpu.VMEM((units, Sk, _LANES), bf16),
            pltpu.VMEM((units, 1, _LANES), f32),
            pltpu.VMEM((_HEADS, rest, Sk), bf16),
            pltpu.VMEM((_HEADS, rest, _LANES), f32),
            pltpu.SMEM((1,), f32),
            per_head((Sk, _LANES), f32, _S_SLOTS),
            per_head((3, half // 2, 2 * third), u32),
            per_head((2, third // 2, half), u32),
            per_head((3, rest // 2, 2 * third), u32),
            per_head((rest, Sk), f32, 2),
            pltpu.VMEM((_HEADS, rest, _LANES), f32),
        ],
        compiler_params=pltpu.CompilerParams(
            dimension_semantics=("arbitrary",),
            vmem_limit_bytes=100 * 1024 * 1024,
            disable_bounds_checks=True,
        ),
    )(qT, kT, vT)
    return jnp.swapaxes(oT.reshape(B, H, D, Sq), 2, 3)
```

```python
import jax
import jax.numpy as jnp
import jax.experimental.pallas as pl
import jax.experimental.pallas.tpu as pltpu
import ml_dtypes
import numpy as np

_HEADS = 8
_LANES = 128
_S_SLOTS = 4


def _dot(a, b):
    return jnp.dot(a, b, preferred_element_type=jnp.float32)


def _dot_t(a, b):
    dims = (((1,), (1,)), ((), ()))
    return jax.lax.dot_general(a, b, dims, preferred_element_type=jnp.float32)


def _fold(x, rows=8):
    return jnp.sum(x.reshape(-1, rows, x.shape[-1]), axis=0)


def _reciprocal(x):
    r = pl.reciprocal(x, approx=True)
    return r + r * (1.0 - x * r)


def _words(x):
    return pltpu.bitcast(x, jnp.uint32)


def _bf16(x):
    return pltpu.bitcast(x, jnp.bfloat16)


@jax.jit
def pallas_standalone__gqa_softmax__near_ridge_kernel(
    q: jax.Array,
    k: jax.Array,
    v: jax.Array,
):
    B, H, Sq, D = q.shape
    Sk = k.shape[2]
    assert k.shape == v.shape == (B, H, Sk, D)
    assert q.dtype == k.dtype == v.dtype == jnp.bfloat16
    f32, bf16, u32 = jnp.float32, jnp.bfloat16, jnp.uint32

    scale = float(np.asarray(D**-0.5, dtype=ml_dtypes.bfloat16))
    log2_scale = scale * float(np.log2(np.e))

    n_blocks = B * H // _HEADS
    tiles, rest = divmod(Sq, _LANES)
    units = _HEADS * tiles
    third, half = D // 3, Sk // 2
    rest_cols = slice(tiles * _LANES, Sq)
    assert D == 192 and Sk == 512 and n_blocks * _HEADS == B * H
    assert tiles >= 6 and rest > 0 and rest % 16 == 0

    def kernel_function(
        q_hbm, k_hbm, v_hbm, o_hbm,
        q_buf, k_buf, v_buf, o_buf, sems, last_sems,
        p_ref, r_ref, rest_p_ref, rest_r_ref, redo_ref,
        s_refs, keys_refs, diff_refs, rest_q_refs, rest_s_refs, rest_m_ref,
    ):
        step = pl.program_id(0)
        q_ref, k_ref = q_buf.at[step % 2], k_buf.at[step % 2]
        v_ref, o_ref = v_buf.at[(step + 1) % 2], o_buf.at[(step + 1) % 2]

        def block(hbm, i):
            return hbm.at[pl.ds(i * _HEADS, _HEADS)]

        def load(n, i):
            hbm, buf = ((k_hbm, k_buf), (q_hbm, q_buf), (v_hbm, v_buf))[n]
            return pltpu.make_async_copy(
                block(hbm, i), buf.at[i % 2], sems.at[n, i % 2]
            )

        def store(i):
            return pltpu.make_async_copy(
                o_buf.at[i % 2], block(o_hbm, i), sems.at[3, i % 2]
            )

        def store_last(g):
            i = n_blocks - 1
            return pltpu.make_async_copy(
                o_buf.at[i % 2, pl.ds(g, 2)],
                o_hbm.at[pl.ds(i * _HEADS + g, 2)],
                last_sems.at[g // 2],
            )

        def query_pairs(h, cols):
            qac = (q_ref[h, :third, cols], q_ref[h, 2 * third :, cols])
            return (
                q_ref[h, third:, cols],
                q_ref[h, : 2 * third, cols],
                jnp.concatenate(qac, 0),
            )

        def put_probs(u, s, m):
            p = jnp.exp2(s - m)
            p_ref[u] = p.astype(bf16)
            r_ref[u] = _reciprocal(jnp.sum(_fold(p, 64), axis=0, keepdims=True))

        def put_rest_probs(h, s_ref):
            m = jnp.max(s_ref[...], axis=1, keepdims=True)
            rest_m_ref[h] = jnp.broadcast_to(m, (rest, _LANES))
            m = jnp.concatenate([rest_m_ref[h]] * (Sk // _LANES), 1)
            p = jnp.exp2(s_ref[...] - m)
            rest_p_ref[h] = p.astype(bf16)
            a, b, c, d = (p[:, j : j + _LANES] for j in range(0, Sk, _LANES))
            total = jnp.sum((a + b) + (c + d), axis=1, keepdims=True)
            rest_r_ref[h] = jnp.broadcast_to(_reciprocal(total), (rest, _LANES))

        def body(do_scores, do_values):
            col_max, unsafe = {}, []

            def prepare(h):
                for j in range(0, half, _LANES):
                    k1a, k1b, k1c, k2a, k2b, k2c = (
                        k_ref[h, d : d + third, j0 : j0 + _LANES]
                        for j0 in (j, half + j)
                        for d in range(0, D, third)
                    )
                    b1, c1, b2, c2 = (x.astype(f32) for x in (k1b, k1c, k2b, k2c))
                    db, dc = b1 - b2, c2 - c1
                    db16, dc16 = db.astype(bf16), dc.astype(bf16)
                    n1 = _fold(jnp.abs(b1) + jnp.abs(c1))
                    n2 = _fold(jnp.abs(b2) + jnp.abs(c2))
                    e1 = _fold(jnp.abs(db - db16.astype(f32)))
                    e2 = _fold(jnp.abs(dc - dc16.astype(f32)))
                    t1, t2 = (
                        jnp.sum(e + 2.0**-20 * other - 2.0**-9 * own, 0, keepdims=True)
                        for e, own, other in ((e1, n1, n2), (e2, n2, n1))
                    )
                    bad = jnp.where((t1 <= 0) & (t2 <= 0), 0.0, 1.0)
                    unsafe.append(jnp.maximum(unsafe.pop(), bad) if unsafe else bad)
                    diff_refs[h][0, :, j : j + _LANES] = _words(db16)
                    diff_refs[h][1, :, j : j + _LANES] = _words(dc16)
                    for n, pair in enumerate(((k2b, k1c), (k1a, db16), (k2a, dc16))):
                        keys_refs[h][n, j // 2 : (j + _LANES) // 2] = _words(
                            jnp.concatenate(pair, 0).T
                        )
                if h == _HEADS - 1:
                    redo_ref[0] = jnp.max(unsafe[0])
                for n, pair in enumerate(query_pairs(h, rest_cols)):
                    rest_q_refs[h][n] = _words(pair.T)

            def scores(u):
                h, t = divmod(u, tiles)
                s_ref, m = s_refs[u % _S_SLOTS], None
                for a, b in ((0, 3 * half // 4), (3 * half // 4, half)):
                    pairs = query_pairs(h, slice(t * _LANES, (t + 1) * _LANES))
                    f5, f1, f2 = (
                        _dot(_bf16(keys_refs[h][n, a // 2 : b // 2]), pairs[n])
                        for n in range(3)
                    )
                    s1, s2 = (f1 + f5) * log2_scale, (f2 + f5) * log2_scale
                    s_ref[a:b] = s1
                    s_ref[half + a : half + b] = s2
                    part = jnp.max(jnp.maximum(s1, s2).reshape(-1, 8, _LANES), axis=0)
                    m = part if m is None else jnp.maximum(m, part)
                col_max[u] = jnp.max(m, axis=0, keepdims=True)

            def probs(u):
                put_probs(u, s_refs[u % _S_SLOTS][...], col_max.pop(u))

            def values(u):
                h, t = divmod(u, tiles)
                o = _dot(v_ref[h], p_ref[u]) * r_ref[u]
                o_ref[h, :, t * _LANES : (t + 1) * _LANES] = o.astype(bf16)

            def rest_scores(h):
                for j in range(0, half, _LANES):
                    one, two = slice(j, j + _LANES), slice(half + j, half + j + _LANES)
                    pairs = (
                        (k_ref[h, third : 2 * third, two], k_ref[h, 2 * third :, one]),
                        (k_ref[h, :third, one], _bf16(diff_refs[h][0, :, one])),
                        (k_ref[h, :third, two], _bf16(diff_refs[h][1, :, one])),
                    )
                    f5, f1, f2 = (
                        _dot(_bf16(rest_q_refs[h][n]), jnp.concatenate(pairs[n], 0))
                        for n in range(3)
                    )
                    rest_s_refs[h % 2][:, one] = (f1 + f5) * log2_scale
                    rest_s_refs[h % 2][:, two] = (f2 + f5) * log2_scale

            def rest_values_low(h):
                o = _dot_t(rest_p_ref[h], v_ref[h, :_LANES]) * rest_r_ref[h]
                o_ref[h, :_LANES, rest_cols] = o.astype(bf16).T

            def rest_values_high(h):
                o = _dot_t(v_ref[h, _LANES:], rest_p_ref[h]) * rest_r_ref[h].T[:1]
                o_ref[h, _LANES:, rest_cols] = o.astype(bf16)

            if do_values:
                values(0)
            if do_scores:
                prepare(0)
            for u in range(units):
                h, t = divmod(u, tiles)
                if do_scores:
                    if t == 2 and h + 1 < _HEADS:
                        prepare(h + 1)
                    scores(u)
                    if u >= 3:
                        probs(u - 3)
                if do_values and u >= 3:
                    values(u - 2)
                    if not do_scores and (h % 2, t) == (0, 1):
                        store_last(h - 2).start()
                for g in (h - h % 2, h - h % 2 + 1):
                    if do_values and (h % 2, t) == (0, 3):
                        rest_values_low(g)
                    if do_values and (h % 2, t) == (0, 5):
                        rest_values_high(g)
                    if do_scores and (h % 2, t) == (1, 2):
                        rest_scores(g)
                    if do_scores and (h % 2, t) == (1, 4):
                        put_rest_probs(g, rest_s_refs[g % 2])
            for u in range(units - 3, units):
                if do_values and u >= units - 2:
                    values(u)
                if do_scores:
                    probs(u)

        @pl.when(step == 0)
        def _():
            load(0, step).start()
            load(1, step).start()

        @pl.when(step < n_blocks)
        def _():
            load(0, step).wait()
            load(1, step).wait()
            load(2, step).start()

        @pl.when(step + 1 < n_blocks)
        def _():
            load(0, step + 1).start()
            load(1, step + 1).start()

        pl.when(step > 0)(lambda: load(2, step - 1).wait())
        pl.when(step > 2)(lambda: store(step - 3).wait())

        pl.when(step == 0)(lambda: body(True, False))
        pl.when((step > 0) & (step < n_blocks))(lambda: body(True, True))

        @pl.when(step == n_blocks)
        def _():
            body(False, True)
            store_last(_HEADS - 2).start()
            if n_blocks > 1:
                store(n_blocks - 2).wait()
            for g in range(0, _HEADS, 2):
                store_last(g).wait()

        pl.when((step > 0) & (step < n_blocks))(lambda: store(step - 1).start())

        @pl.when((redo_ref[0] > 0) & (step < n_blocks))
        def _():
            def redo(h, carry):
                keys = k_ref[h].T
                for t in range(tiles):
                    s = _dot(keys, q_ref[h, :, t * _LANES : (t + 1) * _LANES])
                    s = s * log2_scale
                    put_probs(h * tiles + t, s, jnp.max(s, axis=0, keepdims=True))
                s = _dot(q_ref[h, :, rest_cols].T, k_ref[h])
                rest_s_refs[0][...] = s * log2_scale
                put_rest_probs(h, rest_s_refs[0])
                return carry

            jax.lax.fori_loop(0, _HEADS, redo, 0)

    def buffers(shape, dtype, n=_HEADS):
        return [pltpu.VMEM(shape, dtype) for _ in range(n)]

    qT, kT, vT = (
        jnp.swapaxes(x, 2, 3).reshape(B * H, D, x.shape[2]) for x in (q, k, v)
    )
    oT = pl.pallas_call(
        kernel_function,
        grid=(n_blocks + 1,),
        in_specs=[pl.BlockSpec(memory_space=pl.ANY)] * 3,
        out_specs=pl.BlockSpec(memory_space=pl.ANY),
        out_shape=jax.ShapeDtypeStruct((B * H, D, Sq), q.dtype),
        scratch_shapes=[
            *(pltpu.VMEM((2, _HEADS, D, s), bf16) for s in (Sq, Sk, Sk, Sq)),
            pltpu.SemaphoreType.DMA((4, 2)),
            pltpu.SemaphoreType.DMA((_HEADS // 2,)),
            pltpu.VMEM((units, Sk, _LANES), bf16),
            pltpu.VMEM((units, 1, _LANES), f32),
            pltpu.VMEM((_HEADS, rest, Sk), bf16),
            pltpu.VMEM((_HEADS, rest, _LANES), f32),
            pltpu.SMEM((1,), f32),
            buffers((Sk, _LANES), f32, _S_SLOTS),
            buffers((3, half // 2, 2 * third), u32),
            buffers((2, third // 2, half), u32),
            buffers((3, rest // 2, 2 * third), u32),
            buffers((rest, Sk), f32, 2),
            pltpu.VMEM((_HEADS, rest, _LANES), f32),
        ],
        compiler_params=pltpu.CompilerParams(
            dimension_semantics=("arbitrary",),
            vmem_limit_bytes=100 * 1024 * 1024,
            disable_bounds_checks=True,
        ),
    )(qT, kT, vT)
    return jnp.swapaxes(oT.reshape(B, H, D, Sq), 2, 3)
```
